```python
import os as _os
_os.environ.setdefault("JAX_PLATFORMS", "cpu")
import jax
import jax.numpy as jnp

def _softmax(x, axis=-1):
    return jax.nn.softmax(x, axis=axis)
def _gelu(x):
    return jax.nn.gelu(x, approximate=True)
def _silu(x):
    return jax.nn.silu(x)
def _sigmoid(x):
    return jax.nn.sigmoid(x)
def _layernorm(x, axis=-1, eps=1e-5):
    m = jnp.mean(x, axis=axis, keepdims=True)
    v = jnp.var(x, axis=axis, keepdims=True)
    return (x - m) / jnp.sqrt(v + eps)
def _scatter_add(tgt, idx, src, axis=0):
    return tgt.at[idx].add(src)
def _segment_sum(src, seg, n):
    return jax.ops.segment_sum(src, seg, n)
class _Rng:
    def __init__(self, key):
        self._k = key
    def _next(self):
        self._k, sub = jax.random.split(self._k)
        return sub
    def normal(self, shape):
        return jax.random.normal(self._next(), shape, dtype=jnp.bfloat16)
    def randint(self, lo, hi, shape):
        return jax.random.randint(self._next(), shape, lo, hi, dtype=jnp.int32)
    def uniform(self, shape, lo=0.0, hi=1.0):
        return jax.random.uniform(self._next(), shape, jnp.bfloat16, lo, hi)
    def permutation(self, n):
        return jax.random.permutation(self._next(), n)


kernel_name = 'standalone__gqa_softmax__near_ridge'

def setup_inputs():
    _rng = _Rng(jax.random.key(int.from_bytes(__import__("os").urandom(4), "little")))
    _w = (lambda a: (lambda t: t.astype(jnp.bfloat16) if jnp.issubdtype(t.dtype, jnp.floating) else t)(jnp.asarray(a)))
    B, Hq, Hkv, Sq, Sk, D = 8, 16, 8, 160, 2048, 256
    return {
        "q": _w((lambda *s: _rng.normal(s) * 0.05)(B, Hq, Sq, D)),
        "k": _w((lambda *s: _rng.normal(s) * 3.2)(B, Hkv, Sk, D)),
        "v": _w((lambda *s: _rng.normal(s) * 0.05)(B, Hkv, Sk, D)),
    }

def reference(q, k, v):
    B, Hq, Sq, D = q.shape
    Hkv = k.shape[1]
    rep = Hq // Hkv
    k = jnp.repeat(k, rep, axis=1)
    v = jnp.repeat(v, rep, axis=1)
    scale = D ** -0.5
    scores = jnp.einsum("bhqd,bhkd->bhqk", q, k) * scale
    p = _softmax(scores, axis=-1)
    return jnp.einsum("bhqk,bhkd->bhqd", p, v)
```

```python
import jax, jax.numpy as jnp
import jax.experimental.pallas as pl
import jax.experimental.pallas.tpu as pltpu
LOG2E = 1.4426950408889634

def make(U=8, NB=4, CK=256, DIST=2, LA=1, ND=4, flags="default", vmem=100, nobc=True, JS=0, JO=6, JOW=3, prescale=False, qonce=False, WA=0):
  if flags == "default": flags = {'XLA_TPU_RESCHEDULE_DMA_DONES': True}
  assert U % NB == 0 and DIST < NB
  @jax.jit
  def f(q, k, v):
    B, Hq, Sq, D = q.shape
    _, Hkv, Sk, _ = k.shape
    rep = Hq // Hkv
    M = rep * Sq
    G = B * Hkv
    NC = Sk // CK
    PR = Sk // ND
    CPP = NC // ND
    SPS = 1 + 2 * ND
    c = float(D ** -0.5) * LOG2E
    def kern(q_hbm, k_hbm, v_hbm, o_hbm, q_buf, k_buf, v_buf, o_buf, sems):
        def cp_q(g, slot): return pltpu.make_async_copy(q_hbm.at[g], q_buf[slot], sems.at[slot * SPS])
        def cp_k(g, slot, p): return pltpu.make_async_copy(k_hbm.at[g, pl.ds(p*PR, PR)], k_buf[slot].at[pl.ds(p*PR, PR)], sems.at[slot * SPS + 1 + p])
        def cp_v(g, slot, p): return pltpu.make_async_copy(v_hbm.at[g, pl.ds(p*PR, PR)], v_buf[slot].at[pl.ds(p*PR, PR)], sems.at[slot * SPS + 1 + ND + p])
        def cp_o(g, u): return pltpu.make_async_copy(o_buf[u], o_hbm.at[g], sems.at[NB * SPS + u])
        def start_in(g, slot):
            cp_q(g, slot).start()
            for p in range(ND):
                cp_k(g, slot, p).start()
                cp_v(g, slot, p).start()
        for g in range(DIST):
            start_in(g, g % NB)

        def body(it, carry):
            tasks = [(u, j) for u in range(U) for j in range(NC)]
            n = len(tasks)
            st = {}
            S = {}
            def wait_qk(u, j):
                g = it * U + u
                if j == 0: cp_q(g, u % NB).wait()
                if j % CPP == 0: cp_k(g, u % NB, j // CPP).wait()
            def wait_pv(u, j):
                g = it * U + u
                if j % CPP == 0: cp_v(g, u % NB, j // CPP).wait()
            def qk(u, j):
                slot = u % NB
                qv = q_buf[slot][...]
                if prescale:
                    qv = (qv.astype(jnp.float32) * c).astype(qv.dtype)
                S[(u, j)] = jax.lax.dot_general(qv, k_buf[slot][j*CK:(j+1)*CK, :], (((1,), (1,)), ((), ())), preferred_element_type=jnp.float32)
            def smpv(u, j):
                g = it * U + u
                slot = u % NB
                s = S.pop((u, j))
                def sc(x): return x if prescale else x * c
                mj = jnp.max(s, axis=1, keepdims=True)
                if j == 0:
                    m_new = mj; alpha = None
                else:
                    m_new = jnp.maximum(st['m'], mj)
                    alpha = jnp.exp2(sc(st['m'] - m_new))
                p = jnp.exp2(sc(s - m_new))
                lj = p[:, :128]
                for t in range(1, CK // 128): lj = lj + p[:, t*128:(t+1)*128]
                st['l'] = lj if alpha is None else alpha * st['l'] + lj
                st['m'] = m_new
                if j == JS:
                    @pl.when(g + DIST < G)
                    def _():
                        start_in(g + DIST, (u + DIST) % NB)
                if j == JOW:
                    @pl.when(it > 0)
                    def _():
                        cp_o(g - U, u).wait()
                if j == JO and u > 0:
                    cp_o(g - 1, u - 1).start()
                o = jnp.dot(p.astype(jnp.bfloat16), v_buf[slot][j*CK:(j+1)*CK, :], preferred_element_type=jnp.float32)
                st['o'] = o if alpha is None else alpha * st['o'] + o
                if j == NC - 1:
                    l = jnp.sum(st['l'], axis=1, keepdims=True)
                    o_buf[u][...] = (st['o'] * (1.0 / l)).astype(o_buf[u].dtype)
                    if u == U - 1: cp_o(g, u).start()
            order = []
            for t in range(n + LA):
                if t < n: order.append(('qk', t))
                if t - LA >= 0: order.append(('pv', t - LA))
            waited = -1
            for pos, (kind, t) in enumerate(order):
                while waited < min(pos + WA, len(order) - 1):
                    waited += 1
                    kd, tt = order[waited]
                    (wait_qk if kd == 'qk' else wait_pv)(*tasks[tt])
                (qk if kind == 'qk' else smpv)(*tasks[t])
            return carry
        jax.lax.fori_loop(0, G // U, body, 0)
        for u in range(U):
            cp_o(G - U + u, u).wait()
    out = pl.pallas_call(
        kern,
        in_specs=[pl.BlockSpec(memory_space=pl.ANY)] * 3,
        out_specs=pl.BlockSpec(memory_space=pl.ANY),
        out_shape=jax.ShapeDtypeStruct((G, M, D), q.dtype),
        scratch_shapes=[[pltpu.VMEM((M, D), q.dtype)]*NB, [pltpu.VMEM((Sk, D), k.dtype)]*NB, [pltpu.VMEM((Sk, D), v.dtype)]*NB,
                        [pltpu.VMEM((M, D), q.dtype)]*U,
                        pltpu.SemaphoreType.DMA((NB * SPS + U,))],
        compiler_params=pltpu.CompilerParams(vmem_limit_bytes=vmem*1024*1024, flags=flags, disable_bounds_checks=nobc),
    )(q.reshape(G, M, D), k.reshape(G, Sk, D), v.reshape(G, Sk, D))
    return out.reshape(B, Hq, Sq, D)
  return f


pallas_standalone__gqa_softmax__near_ridge_kernel = make(U=8, ND=2)
```

```python
import jax
import jax.experimental.pallas as pl
import jax.experimental.pallas.tpu as pltpu
import jax.numpy as jnp

_LOG2E = 1.4426950408889634

_CHUNK = 256
_UNROLL = 8
_NBUF = 4
_PREFETCH = 2
_PIECES = 4
_LANES = 128

_AT_PREFETCH = 1
_AT_OUT_WAIT = 5
_AT_OUT_START = 6


@jax.jit
def pallas_standalone__gqa_softmax__near_ridge_kernel(
    q: jax.Array,
    k: jax.Array,
    v: jax.Array,
):
    B, Hq, Sq, D = q.shape
    _, Hkv, Sk, _ = k.shape
    rep = Hq // Hkv
    M = rep * Sq
    G = B * Hkv

    CK = _CHUNK
    NC = Sk // CK
    U, NB, DIST, ND = _UNROLL, _NBUF, _PREFETCH, _PIECES
    PR = Sk // ND
    CPP = NC // ND
    assert Sk % CK == 0 and NC % ND == 0 and G % U == 0 and U % NB == 0
    assert 0 < DIST < NB and D % _LANES == 0 and CK % _LANES == 0
    assert max(_AT_PREFETCH, _AT_OUT_WAIT, _AT_OUT_START) < NC

    c = float(D) ** -0.5 * _LOG2E

    SPS = 1 + 2 * ND
    SEM_OUT = NB * SPS
    SEM_K0 = SEM_OUT + U
    SEM_V0 = SEM_K0 + NC
    NSEM = SEM_V0 + NC

    def kernel(q_hbm, k_hbm, v_hbm, o_hbm, q_buf, k_buf, v_buf, o_buf, sems):
        def cp_q(g, slot):
            return pltpu.make_async_copy(q_hbm.at[g], q_buf[slot], sems.at[slot * SPS])

        def cp_rows(hbm, buf, g, start, size, sem):
            rows = pl.ds(start, size)
            return pltpu.make_async_copy(hbm.at[g, rows], buf.at[rows], sems.at[sem])

        def cp_k(g, slot, p):
            return cp_rows(k_hbm, k_buf[slot], g, p * PR, PR, slot * SPS + 1 + p)

        def cp_v(g, slot, p):
            return cp_rows(v_hbm, v_buf[slot], g, p * PR, PR, slot * SPS + 1 + ND + p)

        def cp_k0(j):
            return cp_rows(k_hbm, k_buf[0], 0, j * CK, CK, SEM_K0 + j)

        def cp_v0(j):
            return cp_rows(v_hbm, v_buf[0], 0, j * CK, CK, SEM_V0 + j)

        def cp_o(g, u):
            return pltpu.make_async_copy(o_buf[u], o_hbm.at[g], sems.at[SEM_OUT + u])

        def start_inputs(g, slot):
            cp_q(g, slot).start()
            for p in range(ND):
                cp_k(g, slot, p).start()
                cp_v(g, slot, p).start()

        cp_q(0, 0).start()
        cp_k0(0).start()
        for j in range(NC):
            if j + 1 < NC:
                cp_k0(j + 1).start()
            cp_v0(j).start()
        for g in range(1, DIST):
            start_inputs(g, g % NB)

        def body(it, carry):
            def wait_piece(cp, cp0, u, j):
                g = it * U + u
                if u == 0:
                    @pl.when(it == 0)
                    def _():
                        cp0(j).wait()

                    if j % CPP == 0:
                        @pl.when(it > 0)
                        def _():
                            cp(g, 0, j // CPP).wait()
                elif j % CPP == 0:
                    cp(g, u % NB, j // CPP).wait()

            scores = {}
            state = {}

            def qk(u, j):
                slot = u % NB
                if j == 0:
                    cp_q(it * U + u, slot).wait()
                wait_piece(cp_k, cp_k0, u, j)
                scores[(u, j)] = jax.lax.dot_general(
                    q_buf[slot][...],
                    k_buf[slot][pl.ds(j * CK, CK), :],
                    (((1,), (1,)), ((), ())),
                    preferred_element_type=jnp.float32,
                )

            def softmax_pv(u, j):
                g = it * U + u
                slot = u % NB
                wait_piece(cp_v, cp_v0, u, j)
                s = scores.pop((u, j))

                m_new = jnp.max(s, axis=1, keepdims=True)
                if j > 0:
                    m_new = jnp.maximum(state["m"], m_new)
                    alpha = jnp.exp2((state["m"] - m_new) * c)
                p = jnp.exp2(s * c - m_new * c)
                l_part = p[:, :_LANES]
                for t in range(1, CK // _LANES):
                    l_part = l_part + p[:, t * _LANES:(t + 1) * _LANES]
                state["l"] = l_part if j == 0 else alpha * state["l"] + l_part
                state["m"] = m_new

                if j == _AT_PREFETCH:
                    @pl.when(g + DIST < G)
                    def _():
                        start_inputs(g + DIST, (u + DIST) % NB)

                if j == _AT_OUT_WAIT:
                    @pl.when(it > 0)
                    def _():
                        cp_o(g - U, u).wait()

                if j == _AT_OUT_START and u > 0:
                    cp_o(g - 1, u - 1).start()

                pv = jnp.dot(
                    p.astype(v_buf[slot].dtype),
                    v_buf[slot][pl.ds(j * CK, CK), :],
                    preferred_element_type=jnp.float32,
                )
                state["o"] = pv if j == 0 else pv + state["o"] * alpha

                if j == NC - 1:
                    l = jnp.sum(state["l"], axis=1, keepdims=True)
                    o_buf[u][...] = (state["o"] * (1.0 / l)).astype(o_buf[u].dtype)
                    if u == U - 1:
                        cp_o(g, u).start()

            tasks = [(u, j) for u in range(U) for j in range(NC)]
            for t in range(len(tasks) + 1):
                if t < len(tasks):
                    qk(*tasks[t])
                if t > 0:
                    softmax_pv(*tasks[t - 1])
            return carry

        jax.lax.fori_loop(0, G // U, body, 0)

        for u in range(U):
            cp_o(G - U + u, u).wait()

    out = pl.pallas_call(
        kernel,
        in_specs=[pl.BlockSpec(memory_space=pl.ANY)] * 3,
        out_specs=pl.BlockSpec(memory_space=pl.ANY),
        out_shape=jax.ShapeDtypeStruct((G, M, D), q.dtype),
        scratch_shapes=[
            [pltpu.VMEM((M, D), q.dtype) for _ in range(NB)],
            [pltpu.VMEM((Sk, D), k.dtype) for _ in range(NB)],
            [pltpu.VMEM((Sk, D), v.dtype) for _ in range(NB)],
            [pltpu.VMEM((M, D), q.dtype) for _ in range(U)],
            pltpu.SemaphoreType.DMA((NSEM,)),
        ],
        compiler_params=pltpu.CompilerParams(
            vmem_limit_bytes=100 * 1024 * 1024,
            disable_bounds_checks=True,
            disable_semaphore_checks=True,
            flags={"XLA_TPU_RESCHEDULE_DMA_DONES": True},
        ),
    )(q.reshape(G, M, D), k.reshape(G, Sk, D), v.reshape(G, Sk, D))
    return out.reshape(B, Hq, Sq, D)
```
